```python
import os as _os
_os.environ.setdefault("JAX_PLATFORMS", "cpu")
import jax
import jax.numpy as jnp

def _softmax(x, axis=-1):
    return jax.nn.softmax(x, axis=axis)
def _gelu(x):
    return jax.nn.gelu(x, approximate=True)
def _silu(x):
    return jax.nn.silu(x)
def _sigmoid(x):
    return jax.nn.sigmoid(x)
def _layernorm(x, axis=-1, eps=1e-5):
    m = jnp.mean(x, axis=axis, keepdims=True)
    v = jnp.var(x, axis=axis, keepdims=True)
    return (x - m) / jnp.sqrt(v + eps)
def _scatter_add(tgt, idx, src, axis=0):
    return tgt.at[idx].add(src)
def _segment_sum(src, seg, n):
    return jax.ops.segment_sum(src, seg, n)
class _Rng:
    def __init__(self, key):
        self._k = key
    def _next(self):
        self._k, sub = jax.random.split(self._k)
        return sub
    def normal(self, shape):
        return jax.random.normal(self._next(), shape, dtype=jnp.bfloat16)
    def randint(self, lo, hi, shape):
        return jax.random.randint(self._next(), shape, lo, hi, dtype=jnp.int32)
    def uniform(self, shape, lo=0.0, hi=1.0):
        return jax.random.uniform(self._next(), shape, jnp.bfloat16, lo, hi)
    def permutation(self, n):
        return jax.random.permutation(self._next(), n)


kernel_name = 'standalone__mha_softmax__near_ridge'

def setup_inputs():
    _rng = _Rng(jax.random.key(int.from_bytes(__import__("os").urandom(4), "little")))
    _w = (lambda a: (lambda t: t.astype(jnp.bfloat16) if jnp.issubdtype(t.dtype, jnp.floating) else t)(jnp.asarray(a)))
    B, H, Sq, Sk, D = 8, 32, 384, 512, 128
    return {
        "q": _w((lambda *s: _rng.normal(s) * 0.4)(B, H, Sq, D)),
        "k": _w((lambda *s: _rng.normal(s) * 0.4)(B, H, Sk, D)),
        "v": _w((lambda *s: _rng.normal(s) * 0.05)(B, H, Sk, D)),
    }

def reference(q, k, v):
    scale = q.shape[-1] ** -0.5
    scores = jnp.einsum("bhqd,bhkd->bhqk", q, k) * scale
    p = _softmax(scores, axis=-1)
    return jnp.einsum("bhqk,bhkd->bhqd", p, v)
```

```python
import jax
import jax.numpy as jnp
import jax.experimental.pallas as pl
import jax.experimental.pallas.tpu as pltpu

_LOG2E = 1.4426950408889634

_G = 8
_LEAD = 2
_NUM, _DEN = 5, 4
_IW = 25


def _head(q, k, v, c):
    s = jax.lax.dot_general(q, k, (((1,), (1,)), ((), ())),
                            preferred_element_type=jnp.float32)
    m = jnp.max(s, axis=-1, keepdims=True)
    p = jnp.exp2((s - m) * c)
    l = jnp.sum(p, axis=-1, keepdims=True)
    o = jnp.dot(p.astype(jnp.bfloat16), v, preferred_element_type=jnp.float32)
    r = pl.reciprocal(l, approx=True)
    r = r * (2.0 - l * r)
    return o * r


@jax.jit
def pallas_standalone__mha_softmax__near_ridge_kernel(
    q: jax.Array,
    k: jax.Array,
    v: jax.Array,
):
    B, H, Sq, D = q.shape
    Sk = k.shape[2]
    BH = B * H
    G = _G
    N = BH // G
    c = (D ** -0.5) * _LOG2E

    def kernel(q_hbm, k_hbm, v_hbm, o_hbm, qb, kb, vb, ob, rsem, wsem):
        def rd(j):
            sl = pl.ds(j * G, G)
            return [pltpu.make_async_copy(q_hbm.at[sl], qb.at[sl], rsem.at[j]),
                    pltpu.make_async_copy(k_hbm.at[sl], kb.at[sl], rsem.at[j]),
                    pltpu.make_async_copy(v_hbm.at[sl], vb.at[sl], rsem.at[j])]

        def issued(i):
            return jnp.minimum(N, _LEAD + ((i + 1) * _NUM + _DEN - 1) // _DEN)

        for j in range(_LEAD):
            for cp in rd(j):
                cp.start()

        def body(i, carry):
            lo = jnp.where(i == 0, _LEAD, issued(i - 1))
            hi = issued(i)

            def issue(j, _):
                for cp in rd(j):
                    cp.start()
                return 0
            jax.lax.fori_loop(lo, hi, issue, 0)

            @pl.when(i < _IW)
            def _():
                for cp in rd(i):
                    cp.wait()

            @pl.when(i == _IW)
            def _():
                def w(j, _):
                    for cp in rd(j):
                        cp.wait()
                    return 0
                jax.lax.fori_loop(_IW, N, w, 0)
                sl = pl.ds(0, _IW * G)
                pltpu.make_async_copy(ob.at[sl], o_hbm.at[sl], wsem).start()

            for g in range(G):
                h = i * G + g
                ob[h] = _head(qb[h], kb[h], vb[h], c).astype(ob.dtype)

            @pl.when(i >= _IW)
            def _():
                sl = pl.ds(i * G, G)
                pltpu.make_async_copy(ob.at[sl], o_hbm.at[sl], wsem).start()
            return carry

        jax.lax.fori_loop(0, N, body, 0)
        pltpu.make_async_copy(ob, o_hbm, wsem).wait()

    q3 = q.reshape(BH, Sq, D)
    k3 = k.reshape(BH, Sk, D)
    v3 = v.reshape(BH, Sk, D)
    out = pl.pallas_call(
        kernel,
        in_specs=[pl.BlockSpec(memory_space=pl.ANY)] * 3,
        out_specs=pl.BlockSpec(memory_space=pl.ANY),
        out_shape=jax.ShapeDtypeStruct((BH, Sq, D), q.dtype),
        scratch_shapes=[
            pltpu.VMEM((BH, Sq, D), q.dtype),
            pltpu.VMEM((BH, Sk, D), k.dtype),
            pltpu.VMEM((BH, Sk, D), v.dtype),
            pltpu.VMEM((BH, Sq, D), q.dtype),
            pltpu.SemaphoreType.DMA((N,)),
            pltpu.SemaphoreType.DMA(()),
        ],
        compiler_params=pltpu.CompilerParams(vmem_limit_bytes=125 * 1024 * 1024),
    )(q3, k3, v3)
    return out.reshape(B, H, Sq, D)
```

```python
import jax
import jax.numpy as jnp
import jax.experimental.pallas as pl
import jax.experimental.pallas.tpu as pltpu

_LOG2E = 1.4426950408889634

_READ_BOUNDS = (1, 2, 3, 4, 5, 6, 8, 10, 12, 14, 17, 20, 23, 26, 32)
_TAIL = 3
_FIRST_WRITES = 20
_PIECE_ROWS = 128


def _attend(q, k, v, c):
    s = jax.lax.dot_general(q, k, (((1,), (1,)), ((), ())),
                            preferred_element_type=jnp.float32)
    m = jnp.max(s, axis=-1, keepdims=True)
    p = jnp.exp2((s - m) * c)
    l = jnp.sum(p, axis=-1, keepdims=True)
    o = jnp.dot(p.astype(v.dtype), v, preferred_element_type=jnp.float32)
    r = pl.reciprocal(l, approx=True)
    r = r * (2.0 - l * r)
    return o * r


@jax.jit
def pallas_standalone__mha_softmax__near_ridge_kernel(
    q: jax.Array,
    k: jax.Array,
    v: jax.Array,
):
    B, H, Sq, D = q.shape
    Sk = k.shape[2]
    c = (D ** -0.5) * _LOG2E

    hi = _READ_BOUNDS
    lo = (0,) + hi[:-1]
    n_chunks = len(hi)
    i_switch = lo[-1]
    n_pieces = Sq // _PIECE_ROWS
    assert hi[-1] == H and Sq % _PIECE_ROWS == 0 and 0 < _TAIL < B
    assert _FIRST_WRITES <= i_switch

    def kernel(q_hbm, k_hbm, v_hbm, o_hbm, qb, kb, vb, ob, rsem, tsem, wsem):
        def read_copies(ci):
            sem = rsem.at[ci]
            sl = pl.ds(lo[ci], hi[ci] - lo[ci])
            cps = [pltpu.make_async_copy(q_hbm.at[:, sl], qb.at[:, sl], sem),
                   pltpu.make_async_copy(k_hbm.at[:, sl], kb.at[:, sl], sem)]
            if ci < n_chunks - 1:
                cps.append(
                    pltpu.make_async_copy(v_hbm.at[:, sl], vb.at[:, sl], sem))
            else:
                slv = pl.ds(lo[ci], hi[ci] - lo[ci] - 1)
                slb = pl.ds(0, B - _TAIL)
                cps.append(
                    pltpu.make_async_copy(v_hbm.at[:, slv], vb.at[:, slv], sem))
                cps.append(
                    pltpu.make_async_copy(v_hbm.at[slb, H - 1],
                                          vb.at[slb, H - 1], sem))
            return cps

        def tail_copy():
            slb = pl.ds(B - _TAIL, _TAIL)
            return pltpu.make_async_copy(v_hbm.at[slb, H - 1],
                                         vb.at[slb, H - 1], tsem)

        def write_copies(i):
            return [
                pltpu.make_async_copy(
                    ob.at[i, r],
                    o_hbm.at[:, i, pl.ds(r * _PIECE_ROWS, _PIECE_ROWS), :],
                    wsem)
                for r in range(n_pieces)
            ]

        def start_writes(first, last):
            def start(i, carry):
                for cp in write_copies(i):
                    cp.start()
                return carry
            jax.lax.fori_loop(first, last, start, 0)

        for ci in range(n_chunks):
            for cp in read_copies(ci):
                cp.start()
        tail_copy().start()

        def step(i, carry):
            for ci in range(n_chunks):
                @pl.when(i == lo[ci])
                def _():
                    for cp in read_copies(ci):
                        cp.wait()
                    if ci == n_chunks - 1:
                        start_writes(0, _FIRST_WRITES)

            @pl.when(i == H - 1)
            def _():
                tail_copy().wait()

            for b in range(B):
                o = _attend(qb[b, i], kb[b, i], vb[b, i], c).astype(ob.dtype)
                for r in range(n_pieces):
                    ob[i, r, b] = o[r * _PIECE_ROWS:(r + 1) * _PIECE_ROWS]

            @pl.when(i == i_switch)
            def _():
                start_writes(_FIRST_WRITES, i_switch + 1)

            @pl.when(i > i_switch)
            def _():
                for cp in write_copies(i):
                    cp.start()

            return carry

        jax.lax.fori_loop(0, H, step, 0)

        def finish(i, carry):
            for cp in write_copies(i):
                cp.wait()
            return carry
        jax.lax.fori_loop(0, H, finish, 0)

    return pl.pallas_call(
        kernel,
        in_specs=[pl.BlockSpec(memory_space=pl.ANY)] * 3,
        out_specs=pl.BlockSpec(memory_space=pl.ANY),
        out_shape=jax.ShapeDtypeStruct((B, H, Sq, D), q.dtype),
        scratch_shapes=[
            pltpu.VMEM((B, H, Sq, D), q.dtype),
            pltpu.VMEM((B, H, Sk, D), k.dtype),
            pltpu.VMEM((B, H, Sk, D), v.dtype),
            pltpu.VMEM((H, n_pieces, B, _PIECE_ROWS, D), q.dtype),
            pltpu.SemaphoreType.DMA((n_chunks,)),
            pltpu.SemaphoreType.DMA(()),
            pltpu.SemaphoreType.DMA(()),
        ],
        compiler_params=pltpu.CompilerParams(
            vmem_limit_bytes=120 * 1024 * 1024),
    )(q, k, v)
```
